```python
import os as _os
_os.environ.setdefault("JAX_PLATFORMS", "cpu")
import jax
import jax.numpy as jnp

def _softmax(x, axis=-1):
    return jax.nn.softmax(x, axis=axis)
def _gelu(x):
    return jax.nn.gelu(x, approximate=True)
def _silu(x):
    return jax.nn.silu(x)
def _sigmoid(x):
    return jax.nn.sigmoid(x)
def _layernorm(x, axis=-1, eps=1e-5):
    m = jnp.mean(x, axis=axis, keepdims=True)
    v = jnp.var(x, axis=axis, keepdims=True)
    return (x - m) / jnp.sqrt(v + eps)
def _scatter_add(tgt, idx, src, axis=0):
    return tgt.at[idx].add(src)
def _segment_sum(src, seg, n):
    return jax.ops.segment_sum(src, seg, n)
class _Rng:
    def __init__(self, key):
        self._k = key
    def _next(self):
        self._k, sub = jax.random.split(self._k)
        return sub
    def normal(self, shape):
        return jax.random.normal(self._next(), shape, dtype=jnp.bfloat16)
    def randint(self, lo, hi, shape):
        return jax.random.randint(self._next(), shape, lo, hi, dtype=jnp.int32)
    def uniform(self, shape, lo=0.0, hi=1.0):
        return jax.random.uniform(self._next(), shape, jnp.bfloat16, lo, hi)
    def permutation(self, n):
        return jax.random.permutation(self._next(), n)


kernel_name = 'recurrent_scan__ssm_conv_s5__mixer_s_mlp__prompt'

def setup_inputs():
    _rng = _Rng(jax.random.key(int.from_bytes(__import__("os").urandom(4), "little")))
    _w = (lambda a: (lambda t: t.astype(jnp.bfloat16) if jnp.issubdtype(t.dtype, jnp.floating) else t)(jnp.asarray(a)))
    def _A_setup():
        B, S, D = 1, 2048, 640
        P = D
        Lambda_re = -0.5 * jnp.exp((lambda *s: _rng.normal(s) * 0.8)(P))
        Lambda_im = (lambda *s: _rng.normal(s) * 0.8)(P) * 1.0
        B_re = (lambda *s: _rng.normal(s) * 0.8)(P, D) * (D ** -0.5)
        B_im = (lambda *s: _rng.normal(s) * 0.8)(P, D) * (D ** -0.5)
        C_re = (lambda *s: _rng.normal(s) * 0.8)(D, P) * (P ** -0.5)
        C_im = (lambda *s: _rng.normal(s) * 0.8)(D, P) * (P ** -0.5)
        log_dt = (lambda *s: _rng.normal(s) * 0.8)(P) * 0.3 - 2.0
        Dskip = (lambda *s: _rng.normal(s) * 0.8)(D)
        return {
            "x": _w((lambda *s: _rng.normal(s) * 0.05)(B, S, D)),
            "Lambda_re": _w(Lambda_re),
            "Lambda_im": _w(Lambda_im),
            "B_re": _w(B_re),
            "B_im": _w(B_im),
            "C_re": _w(C_re),
            "C_im": _w(C_im),
            "log_dt": _w(log_dt),
            "Dskip": _w(Dskip),
        }
    _A_in = _A_setup()

    def _B_setup():
        B, S, D, F = 1, 2048, 640, 1536
        return {
            "x":  _w((lambda *s: _rng.normal(s) * 0.05)(B, S, D)),
            "w1": _w((lambda *s: _rng.normal(s) * 0.8)(D, D) * (D ** -0.5)),
            "w2": _w((lambda *s: _rng.normal(s) * 0.8)(D, D) * (D ** -0.5)),
            "w3": _w((lambda *s: _rng.normal(s) * 0.8)(D, F) * (D ** -0.5)),
            "w4": _w((lambda *s: _rng.normal(s) * 0.8)(F, D) * (F ** -0.5)),
        }
    _B_in = _B_setup()

    return {
        "A_x": _A_in["x"],
        "A_Lambda_re": _A_in["Lambda_re"],
        "A_Lambda_im": _A_in["Lambda_im"],
        "A_B_re": _A_in["B_re"],
        "A_B_im": _A_in["B_im"],
        "A_C_re": _A_in["C_re"],
        "A_C_im": _A_in["C_im"],
        "A_log_dt": _A_in["log_dt"],
        "A_Dskip": _A_in["Dskip"],
        "B_x": _B_in["x"],
        "B_w1": _B_in["w1"],
        "B_w2": _B_in["w2"],
        "B_w3": _B_in["w3"],
        "B_w4": _B_in["w4"],
    }

def reference(A_x, A_Lambda_re, A_Lambda_im, A_B_re, A_B_im, A_C_re, A_C_im, A_log_dt, A_Dskip, B_x, B_w1, B_w2, B_w3, B_w4):
    def _A_ref(x, Lambda_re, Lambda_im, B_re, B_im, C_re, C_im, log_dt, Dskip):
        Bsz, L, H = x.shape
        Lam = Lambda_re + 1j * Lambda_im
        Bmat = B_re + 1j * B_im
        Cmat = C_re + 1j * C_im
        dt = jnp.exp(log_dt)
        Lam_bar = jnp.exp(dt * Lam)
        B_bar = ((Lam_bar - 1.0) / Lam)[:, None] * Bmat
        Bu = jnp.einsum("bld,pd->blp", x + 0j, B_bar)
        h = jnp.zeros_like(Bu[:, 0, :])
        hs = []
        for t in range(L):
            h = Lam_bar[None, :] * h + Bu[:, t, :]
            hs.append(h)
        hseq = jnp.stack(hs, 1)
        y = 2.0 * jnp.einsum("blp,dp->bld", hseq, Cmat).real + x * Dskip[None, None, :]
        return y

    def _B_ref(x, w1, w2, w3, w4):
        B, S, D = x.shape
        h = _gelu(_layernorm(x, axis=-1) @ w1)
        c = D // 4
        g0 = jnp.pad(h[:, :, 0*c:1*c], ((0, 0), (1, 0), (0, 0)))[:, :S, :]
        g1 = jnp.pad(h[:, :, 1*c:2*c], ((0, 0), (0, 1), (0, 0)))[:, 1:, :]
        g2 = jnp.pad(h[:, :, 2*c:3*c], ((0, 0), (2, 0), (0, 0)))[:, :S, :]
        g3 = jnp.pad(h[:, :, 3*c:   ], ((0, 0), (0, 2), (0, 0)))[:, 2:, :]
        hs = jnp.concatenate([g0, g1, g2, g3], axis=-1) @ w2
        x1 = x + hs
        h2 = _gelu(_layernorm(x1, axis=-1) @ w3) @ w4
        return x1 + h2

    x = A_x
    xn = _layernorm(x, axis=-1)
    s = _A_ref(xn, A_Lambda_re, A_Lambda_im, A_B_re, A_B_im, A_C_re, A_C_im, A_log_dt, A_Dskip)
    g = _silu(_B_ref(xn, B_w1, B_w2, B_w3, B_w4))
    return x + s * g
```

```python
import functools
import jax
import jax.numpy as jnp
from jax import lax
import jax.experimental.pallas as pl
import jax.experimental.pallas.tpu as pltpu

S = 2048
D = 640
P = 640
F = 1536
T = 256
NSTEP = S // T
NSEG = 8
SEG = T // NSEG
EPS = 1e-5
f32 = jnp.float32
bf16 = jnp.bfloat16

ORDER_FIRST = "W2 Bre W3 W4 W10 Bim w2 fa V3 scan fb W7 w3 W8 w4 W5 W6 fix Cprep C final W9".split()
ORDER_MID = "Bre fa Bim w2 V3 fb scan fix w3 C w4 final".split()
ORDER_LAST = "Bre Bim w2 V3 scan fix w3 C w4 final".split()
RAWC = 0
DMA_ORDER = [int(v) for v in "0 1 2 3 4 10 7 8 5 6 9".split()]


def _ln(v):
    m = jnp.mean(v, axis=-1, keepdims=True)
    c = v - m
    var = jnp.mean(c * c, axis=-1, keepdims=True)
    return c * lax.rsqrt(var + EPS)


def _gelu(v):
    return jax.nn.gelu(v, approximate=True)


def _nt(a, b):
    return lax.dot_general(a, b, (((1,), (1,)), ((), ())), preferred_element_type=f32)


def _nn(a, b):
    return jnp.dot(a, b, preferred_element_type=f32)


def _cmul(ar, ai, br, bi):
    return ar * br - ai * bi, ar * bi + ai * br


def _transpose8(V, sub):
    for d in (1, 2, 4):
        mask = (sub & d) == 0
        nv = list(V)
        for a in range(8):
            if a & d == 0:
                b = a + d
                nv[a] = jnp.where(mask, V[a], pltpu.roll(V[b], d, 0))
                nv[b] = jnp.where(mask, pltpu.roll(V[a], 8 - d, 0), V[b])
        V = nv
    return V


def kernel(lre_h, lim_h, ldt_h, dsk_h,
           x_hbm, bre_hbm, bim_hbm, cre_hbm, cim_hbm, w1_hbm, w2_hbm, w3_hbm, w4_hbm,
           o_hbm,
           x_v, bre, bim, cre, cim, w1, w2, w3, w4, sems,
           cst, powre, powim, lamc, carry, xP_s, xn_s, bu_s, hext_s, xp_s, o_s, osems, g_s, lre_r, lim_r, ldt_r, dsk_r, vsems):
    i = pl.program_id(0)

    XA = T + 16
    X0 = 2 * T + 16
    copies = [
        pltpu.make_async_copy(x_hbm.at[pl.ds(0, XA)], x_v.at[pl.ds(0, XA)], sems.at[0]),
        pltpu.make_async_copy(w1_hbm, w1, sems.at[1]),
        pltpu.make_async_copy(bre_hbm, bre, sems.at[2]),
        pltpu.make_async_copy(bim_hbm, bim, sems.at[3]),
        pltpu.make_async_copy(w2_hbm, w2, sems.at[4]),
        pltpu.make_async_copy(cre_hbm, cre, sems.at[5]),
        pltpu.make_async_copy(cim_hbm, cim, sems.at[6]),
        pltpu.make_async_copy(w3_hbm, w3, sems.at[7]),
        pltpu.make_async_copy(w4_hbm, w4, sems.at[8]),
        pltpu.make_async_copy(x_hbm.at[pl.ds(X0, S - X0)], x_v.at[pl.ds(X0, S - X0)], sems.at[9]),
        pltpu.make_async_copy(x_hbm.at[pl.ds(XA, X0 - XA)], x_v.at[pl.ds(XA, X0 - XA)], sems.at[10]),
    ]

    vcopies = [pltpu.make_async_copy(a, b, vsems.at[k])
               for k, (a, b) in enumerate(((lre_h, lre_r), (lim_h, lim_r), (ldt_h, ldt_r), (dsk_h, dsk_r)))]

    def out_copies(step, slot):
        return [pltpu.make_async_copy(o_s.at[slot, :, k, :], o_hbm.at[step, k], osems.at[slot * NSEG + k])
                for k in range(NSEG)]

    def row(ref):
        return ref[...].astype(f32).reshape(1, P)

    def front_a(j, slot):
        sub = lax.broadcasted_iota(jnp.int32, (8, D), 0)
        t0 = pl.multiple_of(j * T, T)
        xf = x_v[pl.ds(t0, T), :].astype(f32)
        W = []
        for g in range(SEG // 8):
            W += _transpose8([xf[a * SEG + g * 8:a * SEG + g * 8 + 8] for a in range(NSEG)], sub)
        ps = pl.multiple_of(jnp.maximum(t0 - 16, 0), 16)
        ns = pl.multiple_of(jnp.minimum(t0 + T, S - 16), 16)
        xp = x_v[pl.ds(ps, 16), :].astype(f32)[8:16]
        xq = x_v[pl.ds(ns, 16), :].astype(f32)[0:8]
        xe = jnp.concatenate(W + [xp, xq], axis=0)
        xP_s[slot] = xe[0:T]
        xne = _ln(xe)
        xn_s[slot] = xne[0:T]
        xp_s[slot] = xne[0:T].astype(bf16)
        return _ln(xne).astype(bf16)

    def front_b(j, lnb):
        sub = lax.broadcasted_iota(jnp.int32, (8, D), 0)
        h1 = _nn(lnb, w1[...])
        hp = jnp.where(j > 0, h1[T:T + 8], 0.0)
        hq = jnp.where(j < NSTEP - 1, h1[T + 8:T + 16], 0.0)
        m0 = h1[0:8]
        m1 = h1[8:16]
        m30 = h1[T - 16:T - 8]
        m31 = h1[T - 8:T]
        hext_s[0:8, :] = jnp.where(sub == 0, pltpu.roll(hp, 2, 0), pltpu.roll(m30, 1, 0))
        hext_s[8:16, :] = jnp.where(sub == 0, pltpu.roll(hp, 1, 0), pltpu.roll(m31, 1, 0))
        hext_s[16:16 + T, :] = h1[0:T]
        hext_s[16 + T:24 + T, :] = jnp.where(sub == 7, pltpu.roll(hq, 7, 0), pltpu.roll(m0, 7, 0))
        hext_s[24 + T:32 + T, :] = jnp.where(sub == 7, pltpu.roll(hq, 6, 0), pltpu.roll(m1, 7, 0))
        lane = lax.broadcasted_iota(jnp.int32, (T, 128), 1)
        a1 = hext_s[8:8 + T, 0:256]
        a2 = hext_s[24:24 + T, 128:384]
        a3 = hext_s[0:T, 256:512]
        a4 = hext_s[32:32 + T, 384:640]
        g_s[...] = _gelu(jnp.concatenate([
            a1[:, 0:128],
            jnp.where(lane < 32, a1[:, 128:256], a2[:, 0:128]),
            jnp.where(lane < 64, a2[:, 128:256], a3[:, 0:128]),
            jnp.where(lane < 96, a3[:, 128:256], a4[:, 0:128]),
            a4[:, 128:256],
        ], axis=1)).astype(bf16)

    def init_params():
        lr = row(lre_r)
        li = row(lim_r)
        dt = jnp.exp(row(ldt_r))
        dlr = dt * lr
        dli = dt * li
        e = (lax.broadcasted_iota(jnp.int32, (8, P), 0) + 1).astype(f32)
        mag = jnp.exp(e * dlr)
        ang = e * dli
        pr = mag * jnp.cos(ang)
        pi_ = mag * jnp.sin(ang)
        n = 8
        while n < SEG:
            qr, qi = _cmul(pr, pi_, pr[n - 1:n], pi_[n - 1:n])
            pr = jnp.concatenate([pr, qr], axis=0)
            pi_ = jnp.concatenate([pi_, qi], axis=0)
            n *= 2
        for t in range(SEG):
            powre[t * 8:(t + 1) * 8, :] = jnp.broadcast_to(pr[t:t + 1], (8, P))
            powim[t * 8:(t + 1) * 8, :] = jnp.broadcast_to(pi_[t:t + 1], (8, P))
        lamc[0] = jnp.broadcast_to(pr[0:1], (8, P))
        lamc[1] = jnp.broadcast_to(pi_[0:1], (8, P))
        ar, ai = pr[SEG - 1:SEG], pi_[SEG - 1:SEG]
        for k in range(3):
            lamc[2 + 2 * k] = jnp.broadcast_to(ar, (8, P))
            lamc[3 + 2 * k] = jnp.broadcast_to(ai, (8, P))
            ar, ai = _cmul(ar, ai, ar, ai)
        carry[...] = jnp.zeros_like(carry)
        nr = pr[0:1] - 1.0
        ni = pi_[0:1]
        den = lr * lr + li * li
        cr = (nr * lr + ni * li) / den
        ci = (ni * lr - nr * li) / den
        return cr, ci

    def body(first, last):
        slot = i % 2
        st = {}
        if first:
            for cp in vcopies:
                cp.start()
            for k in DMA_ORDER[:2]:
                copies[k].start()
            for cp in vcopies:
                cp.wait()
            for k in DMA_ORDER[2:]:
                copies[k].start()
            st['cr'], st['ci'] = init_params()
            copies[0].wait()
            copies[1].wait()
            front_b(0, front_a(0, 0))

        def s_Bre():
            bu_s[:, 0:P] = _nt(xp_s[slot], bre[...])

        def s_Bim():
            bu_s[:, P:2 * P] = _nt(xp_s[slot], bim[...])

        def s_fa():
            st['lnb'] = front_a(i + 1, 1 - slot)

        def s_fb():
            front_b(i + 1, st['lnb'])

        def s_w2():
            st['hs'] = _nn(g_s[...], w2[...])

        def s_V3():
            st['xn'] = xn_s[slot]
            st['x1'] = st['xn'] + st['hs']
            st['ln1'] = _ln(st['x1']).astype(bf16)

        def s_w3():
            st['h3'] = _gelu(_nn(st['ln1'], w3[...])).astype(bf16)

        def s_scan():
            lr = lamc[0]
            li = lamc[1]
            hr = carry[0]
            hi = carry[1]
            for t in range(SEG):
                br = bu_s[t * 8:(t + 1) * 8, 0:P]
                bi = bu_s[t * 8:(t + 1) * 8, P:2 * P]
                nhr = lr * hr - li * hi + br
                nhi = lr * hi + li * hr + bi
                hr, hi = nhr, nhi
                bu_s[t * 8:(t + 1) * 8, 0:P] = hr
                bu_s[t * 8:(t + 1) * 8, P:2 * P] = hi
            sub = lax.broadcasted_iota(jnp.int32, (8, P), 0)
            gr, gi = hr, hi
            for k, sh in enumerate((1, 2, 4)):
                ar = lamc[2 + 2 * k]
                ai = lamc[3 + 2 * k]
                sr = jnp.where(sub >= sh, pltpu.roll(gr, sh, 0), 0.0)
                si = jnp.where(sub >= sh, pltpu.roll(gi, sh, 0), 0.0)
                gr, gi = gr + ar * sr - ai * si, gi + ar * si + ai * sr
            rr = pltpu.roll(gr, 1, 0)
            ri = pltpu.roll(gi, 1, 0)
            carry[0] = jnp.where(sub == 0, rr, 0.0)
            carry[1] = jnp.where(sub == 0, ri, 0.0)
            st['gpr'] = jnp.where(sub >= 1, rr, 0.0)[None]
            st['gpi'] = jnp.where(sub >= 1, ri, 0.0)[None]

        def s_fix():
            gpr, gpi = st['gpr'], st['gpi']
            pr = powre[...].reshape(SEG, 8, P)
            pi_ = powim[...].reshape(SEG, 8, P)
            hlr = bu_s[:, 0:P].reshape(SEG, 8, P)
            hli = bu_s[:, P:2 * P].reshape(SEG, 8, P)
            hfr = (hlr + pr * gpr - pi_ * gpi).reshape(T, P)
            hfi = (hli + pr * gpi + pi_ * gpr).reshape(T, P)
            if first and RAWC:
                c2r = 2.0 * st['cr']
                c2i = 2.0 * st['ci']
                st['qr'] = (hfr * c2r - hfi * c2i).astype(bf16)
                st['qi'] = (-(hfr * c2i + hfi * c2r)).astype(bf16)
            else:
                st['hcat'] = jnp.concatenate([hfr.astype(bf16), hfi.astype(bf16)], axis=1)

        def s_Cprep():
            cr, ci = st['cr'], st['ci']
            c_r = cre[...].astype(f32)
            c_i = cim[...].astype(f32)
            cst[:, 0:P] = (2.0 * (c_r * cr - c_i * ci)).astype(bf16)
            cst[:, P:2 * P] = (-2.0 * (c_r * ci + c_i * cr)).astype(bf16)

        def s_C():
            if first and RAWC:
                st['y'] = _nt(st['qr'], cre[...]) + _nt(st['qi'], cim[...])
            else:
                st['y'] = _nt(st['hcat'], cst[...])

        def s_w4():
            st['h2'] = _nn(st['h3'], w4[...])

        def s_final():
            z = st['x1'] + st['h2']
            gate = z * jax.nn.sigmoid(z)
            s = st['y'] + st['xn'] * row(dsk_r)
            o_s[slot] = (xP_s[slot] + s * gate).reshape(SEG, NSEG, D)

        stages = dict(Bre=s_Bre, Bim=s_Bim, fa=s_fa, fb=s_fb, w2=s_w2, V3=s_V3, w3=s_w3, scan=s_scan,
                      Cprep=s_Cprep, fix=s_fix, C=s_C, w4=s_w4, final=s_final)
        order = ORDER_FIRST if first else (ORDER_LAST if last else ORDER_MID)
        for name in order:
            if name[0] == 'W':
                copies[int(name[1:])].wait()
            else:
                stages[name]()

        for cp in out_copies(i, slot):
            cp.start()
        if last:
            for cp in out_copies(i - 1, 1 - slot):
                cp.wait()
            for cp in out_copies(i, slot):
                cp.wait()

    @pl.when(i >= 2)
    def _():
        for cp in out_copies(i - 2, i % 2):
            cp.wait()

    @pl.when(i == 0)
    def _():
        with jax.named_scope("first"):
            body(True, False)

    @pl.when(jnp.logical_and(i > 0, i < NSTEP - 1))
    def _():
        with jax.named_scope("mid"):
            body(False, False)

    @pl.when(i == NSTEP - 1)
    def _():
        with jax.named_scope("last"):
            body(False, True)


@jax.jit
def pallas_recurrent_scan__ssm_conv_s5__mixer_s_mlp__prompt_kernel(
    A_x, A_Lambda_re, A_Lambda_im, A_B_re, A_B_im, A_C_re, A_C_im, A_log_dt, A_Dskip,
    B_x, B_w1, B_w2, B_w3, B_w4,
):
    x = A_x.reshape(S, D)
    vec = pl.BlockSpec((P,), lambda i: (0,))
    anyspec = pl.BlockSpec(memory_space=pl.ANY)
    out = pl.pallas_call(
        kernel,
        grid=(NSTEP,),
        in_specs=[anyspec] * 13,
        out_specs=anyspec,
        out_shape=jax.ShapeDtypeStruct((NSTEP, NSEG, SEG, D), f32),
        scratch_shapes=[
            pltpu.VMEM((S, D), bf16),
            pltpu.VMEM((P, D), bf16),
            pltpu.VMEM((P, D), bf16),
            pltpu.VMEM((D, P), bf16),
            pltpu.VMEM((D, P), bf16),
            pltpu.VMEM((D, D), bf16),
            pltpu.VMEM((D, D), bf16),
            pltpu.VMEM((D, F), bf16),
            pltpu.VMEM((F, D), bf16),
            pltpu.SemaphoreType.DMA((11,)),
            pltpu.VMEM((D, 2 * P), bf16),
            pltpu.VMEM((T, P), f32),
            pltpu.VMEM((T, P), f32),
            pltpu.VMEM((8, 8, P), f32),
            pltpu.VMEM((2, 8, P), f32),
            pltpu.VMEM((2, T, D), f32),
            pltpu.VMEM((2, T, D), f32),
            pltpu.VMEM((T, 2 * P), f32),
            pltpu.VMEM((T + 32, D), f32),
            pltpu.VMEM((2, T, D), bf16),
            pltpu.VMEM((2, SEG, NSEG, D), f32),
            pltpu.SemaphoreType.DMA((2 * NSEG,)),
            pltpu.VMEM((T, D), bf16),
            pltpu.VMEM((P,), bf16),
            pltpu.VMEM((P,), bf16),
            pltpu.VMEM((P,), bf16),
            pltpu.VMEM((P,), bf16),
            pltpu.SemaphoreType.DMA((4,)),
        ],
        compiler_params=pltpu.CompilerParams(
            dimension_semantics=("arbitrary",),
            vmem_limit_bytes=100 * 1024 * 1024,
        ),
    )(A_Lambda_re, A_Lambda_im, A_log_dt, A_Dskip,
      x, A_B_re, A_B_im, A_C_re, A_C_im, B_w1, B_w2, B_w3, B_w4)
    return out.reshape(1, S, D)
```

```python
import jax
import jax.numpy as jnp
from jax import lax
import jax.experimental.pallas as pl
import jax.experimental.pallas.tpu as pltpu

S = 2048
D = 640
P = 640
F = 1536
T = 256
NSTEP = S // T
NSEG = 8
SEG = T // NSEG
EPS = 1e-5
f32 = jnp.float32
bf16 = jnp.bfloat16


ORDER_FIRST = "W4 W2 w2 Bre V3 W3 W10 Bim fa fb scan W7 w3 W8 w4 W5 W6 fix Cprep C final W9".split()
ORDER_MID = "Bre fa Bim w2 V3 fb scan fix w3 C w4 final".split()
ORDER_LAST = "w2 Bim Bre scan V3 w3 fix C w4 final".split()
DMA_ORDER = (0, 1, 4, 2, 3, 10, 7, 8, 5, 6, 9)


def _ln(v):
    m = jnp.mean(v, axis=-1, keepdims=True)
    c = v - m
    var = jnp.mean(c * c, axis=-1, keepdims=True)
    return c * lax.rsqrt(var + EPS)


def _gelu(v):
    return jax.nn.gelu(v, approximate=True)


def _nt(a, b):
    return lax.dot_general(a, b, (((1,), (1,)), ((), ())), preferred_element_type=f32)


def _nn(a, b):
    return jnp.dot(a, b, preferred_element_type=f32)


def _cmul(ar, ai, br, bi):
    return ar * br - ai * bi, ar * bi + ai * br


def _transpose8(V, sub):
    for d in (1, 2, 4):
        mask = (sub & d) == 0
        nv = list(V)
        for a in range(8):
            if a & d == 0:
                b = a + d
                nv[a] = jnp.where(mask, V[a], pltpu.roll(V[b], d, 0))
                nv[b] = jnp.where(mask, pltpu.roll(V[a], 8 - d, 0), V[b])
        V = nv
    return V


def _kernel(lre_h, lim_h, ldt_h, dsk_h,
            x_hbm, bre_hbm, bim_hbm, cre_hbm, cim_hbm, w1_hbm, w2_hbm, w3_hbm, w4_hbm,
            o_hbm,
            x_v, bre, bim, cre, cim, w1, w2, w3, w4, sems,
            cst, powre, powim, lamc, carry, xP_s, xn_s, bu_s, hext_s, xp_s, o_s, osems, g_s,
            lre_r, lim_r, ldt_r, dsk_r, vsems):
    i = pl.program_id(0)

    XA = T + 16
    X0 = 2 * T + 16
    copies = [
        pltpu.make_async_copy(x_hbm.at[pl.ds(0, XA)], x_v.at[pl.ds(0, XA)], sems.at[0]),
        pltpu.make_async_copy(w1_hbm, w1, sems.at[1]),
        pltpu.make_async_copy(bre_hbm, bre, sems.at[2]),
        pltpu.make_async_copy(bim_hbm, bim, sems.at[3]),
        pltpu.make_async_copy(w2_hbm, w2, sems.at[4]),
        pltpu.make_async_copy(cre_hbm, cre, sems.at[5]),
        pltpu.make_async_copy(cim_hbm, cim, sems.at[6]),
        pltpu.make_async_copy(w3_hbm, w3, sems.at[7]),
        pltpu.make_async_copy(w4_hbm, w4, sems.at[8]),
        pltpu.make_async_copy(x_hbm.at[pl.ds(X0, S - X0)], x_v.at[pl.ds(X0, S - X0)], sems.at[9]),
        pltpu.make_async_copy(x_hbm.at[pl.ds(XA, X0 - XA)], x_v.at[pl.ds(XA, X0 - XA)], sems.at[10]),
    ]
    vcopies = [pltpu.make_async_copy(a, b, vsems.at[k])
               for k, (a, b) in enumerate(((lre_h, lre_r), (lim_h, lim_r), (ldt_h, ldt_r), (dsk_h, dsk_r)))]

    def out_start(step, slot):
        for k in range(NSEG):
            pltpu.make_async_copy(o_s.at[slot, :, k, :], o_hbm.at[step, k], osems.at[slot]).start()

    def out_wait(step, slot):
        pltpu.make_async_copy(o_hbm.at[step], o_hbm.at[step], osems.at[slot]).wait()

    def row(ref):
        return ref[...].astype(f32).reshape(1, P)

    def front_a(j, slot):
        sub = lax.broadcasted_iota(jnp.int32, (8, D), 0)
        t0 = pl.multiple_of(j * T, T)
        xu = pltpu.bitcast(x_v[pl.ds(t0, T), :], jnp.uint32)
        hs = SEG // 2
        W = []
        for g in range(hs // 8):
            for w in _transpose8([xu[a * hs + g * 8:a * hs + g * 8 + 8] for a in range(NSEG)], sub):
                W.append(pltpu.bitcast(w << 16, f32))
                W.append(pltpu.bitcast(w & jnp.uint32(0xFFFF0000), f32))
        ps = pl.multiple_of(jnp.maximum(t0 - 16, 0), 16)
        ns = pl.multiple_of(jnp.minimum(t0 + T, S - 16), 16)
        xp = x_v[pl.ds(ps, 16), :].astype(f32)[8:16]
        xq = x_v[pl.ds(ns, 16), :].astype(f32)[0:8]
        xe = jnp.concatenate(W + [xp, xq], axis=0)
        xP_s[slot] = xe[0:T]
        xne = _ln(xe)
        xn_s[slot] = xne[0:T]
        xp_s[slot] = xne[0:T].astype(bf16)
        return _ln(xne).astype(bf16)

    def front_b(j, lnb):
        sub = lax.broadcasted_iota(jnp.int32, (8, D), 0)
        h1 = _nn(lnb, w1[...])
        hp = jnp.where(j > 0, h1[T:T + 8], 0.0)
        hq = jnp.where(j < NSTEP - 1, h1[T + 8:T + 16], 0.0)
        m0 = h1[0:8]
        m1 = h1[8:16]
        m30 = h1[T - 16:T - 8]
        m31 = h1[T - 8:T]
        hext_s[0:8, :] = jnp.where(sub == 0, pltpu.roll(hp, 2, 0), pltpu.roll(m30, 1, 0))
        hext_s[8:16, :] = jnp.where(sub == 0, pltpu.roll(hp, 1, 0), pltpu.roll(m31, 1, 0))
        hext_s[16:16 + T, :] = h1[0:T]
        hext_s[16 + T:24 + T, :] = jnp.where(sub == 7, pltpu.roll(hq, 7, 0), pltpu.roll(m0, 7, 0))
        hext_s[24 + T:32 + T, :] = jnp.where(sub == 7, pltpu.roll(hq, 6, 0), pltpu.roll(m1, 7, 0))
        lane = lax.broadcasted_iota(jnp.int32, (T, 128), 1)
        a1 = hext_s[8:8 + T, 0:256]
        a2 = hext_s[24:24 + T, 128:384]
        a3 = hext_s[0:T, 256:512]
        a4 = hext_s[32:32 + T, 384:640]
        g_s[...] = _gelu(jnp.concatenate([
            a1[:, 0:128],
            jnp.where(lane < 32, a1[:, 128:256], a2[:, 0:128]),
            jnp.where(lane < 64, a2[:, 128:256], a3[:, 0:128]),
            jnp.where(lane < 96, a3[:, 128:256], a4[:, 0:128]),
            a4[:, 128:256],
        ], axis=1)).astype(bf16)

    def init_params():
        lr = row(lre_r)
        li = row(lim_r)
        dt = jnp.exp(row(ldt_r)).astype(bf16).astype(f32)
        dlr = dt * lr
        dli = dt * li
        e = (lax.broadcasted_iota(jnp.int32, (8, P), 0) + 1).astype(f32)
        mag = jnp.exp(e * dlr)
        ang = e * dli
        pr = mag * jnp.cos(ang)
        pi_ = mag * jnp.sin(ang)
        n = 8
        while n < SEG:
            qr, qi = _cmul(pr, pi_, pr[n - 1:n], pi_[n - 1:n])
            pr = jnp.concatenate([pr, qr], axis=0)
            pi_ = jnp.concatenate([pi_, qi], axis=0)
            n *= 2
        for t in range(SEG):
            powre[t * 8:(t + 1) * 8, :] = jnp.broadcast_to(pr[t:t + 1], (8, P))
            powim[t * 8:(t + 1) * 8, :] = jnp.broadcast_to(pi_[t:t + 1], (8, P))
        lamc[0] = jnp.broadcast_to(pr[0:1], (8, P))
        lamc[1] = jnp.broadcast_to(pi_[0:1], (8, P))
        ar, ai = pr[SEG - 1:SEG], pi_[SEG - 1:SEG]
        for k in range(3):
            lamc[2 + 2 * k] = jnp.broadcast_to(ar, (8, P))
            lamc[3 + 2 * k] = jnp.broadcast_to(ai, (8, P))
            ar, ai = _cmul(ar, ai, ar, ai)
        carry[...] = jnp.zeros_like(carry)
        nr = pr[0:1] - 1.0
        ni = pi_[0:1]
        den = lr * lr + li * li
        cr = (nr * lr + ni * li) / den
        ci = (ni * lr - nr * li) / den
        return cr, ci

    def body(first, last):
        slot = i % 2
        st = {}
        if first:
            for cp in vcopies:
                cp.start()
            for k in DMA_ORDER[:2]:
                copies[k].start()
            for cp in vcopies:
                cp.wait()
            for k in DMA_ORDER[2:]:
                copies[k].start()
            st['cr'], st['ci'] = init_params()
            copies[0].wait()
            copies[1].wait()
            front_b(0, front_a(0, 0))

        def s_Bre():
            bu_s[:, 0:P] = _nt(xp_s[slot], bre[...])

        def s_Bim():
            bu_s[:, P:2 * P] = _nt(xp_s[slot], bim[...])

        def s_fa():
            st['lnb'] = front_a(i + 1, 1 - slot)

        def s_fb():
            front_b(i + 1, st['lnb'])

        def s_w2():
            st['hs'] = _nn(g_s[...], w2[...])

        def s_V3():
            st['xn'] = xn_s[slot]
            st['x1'] = st['xn'] + st['hs']
            st['ln1'] = _ln(st['x1']).astype(bf16)

        def s_w3():
            st['h3'] = _gelu(_nn(st['ln1'], w3[...])).astype(bf16)

        def s_scan():
            lr = lamc[0]
            li = lamc[1]
            hr = carry[0]
            hi = carry[1]
            for t in range(SEG):
                br = bu_s[t * 8:(t + 1) * 8, 0:P]
                bi = bu_s[t * 8:(t + 1) * 8, P:2 * P]
                nhr = lr * hr - li * hi + br
                nhi = lr * hi + li * hr + bi
                hr, hi = nhr, nhi
                bu_s[t * 8:(t + 1) * 8, 0:P] = hr
                bu_s[t * 8:(t + 1) * 8, P:2 * P] = hi
            sub = lax.broadcasted_iota(jnp.int32, (8, P), 0)
            gr, gi = hr, hi
            for k, sh in enumerate((1, 2, 4)):
                ar = lamc[2 + 2 * k]
                ai = lamc[3 + 2 * k]
                sr = jnp.where(sub >= sh, pltpu.roll(gr, sh, 0), 0.0)
                si = jnp.where(sub >= sh, pltpu.roll(gi, sh, 0), 0.0)
                gr, gi = gr + ar * sr - ai * si, gi + ar * si + ai * sr
            rr = pltpu.roll(gr, 1, 0)
            ri = pltpu.roll(gi, 1, 0)
            carry[0] = jnp.where(sub == 0, rr, 0.0)
            carry[1] = jnp.where(sub == 0, ri, 0.0)
            st['gpr'] = jnp.where(sub >= 1, rr, 0.0)[None]
            st['gpi'] = jnp.where(sub >= 1, ri, 0.0)[None]

        def s_fix():
            gpr, gpi = st['gpr'], st['gpi']
            pr = powre[...].reshape(SEG, 8, P)
            pi_ = powim[...].reshape(SEG, 8, P)
            hlr = bu_s[:, 0:P].reshape(SEG, 8, P)
            hli = bu_s[:, P:2 * P].reshape(SEG, 8, P)
            hfr = (hlr + pr * gpr - pi_ * gpi).reshape(T, P)
            hfi = (hli + pr * gpi + pi_ * gpr).reshape(T, P)
            st['hcat'] = jnp.concatenate([hfr.astype(bf16), hfi.astype(bf16)], axis=1)

        def s_Cprep():
            cr, ci = st['cr'], st['ci']
            c_r = cre[...].astype(f32)
            c_i = cim[...].astype(f32)
            cst[:, 0:P] = (2.0 * (c_r * cr - c_i * ci)).astype(bf16)
            cst[:, P:2 * P] = (-2.0 * (c_r * ci + c_i * cr)).astype(bf16)

        def s_C():
            st['y'] = _nt(st['hcat'], cst[...])

        def s_w4():
            st['h2'] = _nn(st['h3'], w4[...])

        def s_final():
            z = st['x1'] + st['h2']
            gate = z * jax.nn.sigmoid(z)
            s = st['y'] + st['xn'] * row(dsk_r)
            o_s[slot] = (xP_s[slot] + s * gate).reshape(SEG, NSEG, D)

        stages = dict(Bre=s_Bre, Bim=s_Bim, fa=s_fa, fb=s_fb, w2=s_w2, V3=s_V3, w3=s_w3, scan=s_scan,
                      Cprep=s_Cprep, fix=s_fix, C=s_C, w4=s_w4, final=s_final)
        order = ORDER_FIRST if first else (ORDER_LAST if last else ORDER_MID)
        for name in order:
            if name[0] == 'W':
                copies[int(name[1:])].wait()
            else:
                stages[name]()

        out_start(i, slot)
        if last:
            out_wait(i - 1, 1 - slot)
            out_wait(i, slot)

    @pl.when(i >= 2)
    def _():
        out_wait(i - 2, i % 2)

    @pl.when(i == 0)
    def _():
        body(True, False)

    @pl.when(jnp.logical_and(i > 0, i < NSTEP - 1))
    def _():
        body(False, False)

    @pl.when(i == NSTEP - 1)
    def _():
        body(False, True)


@jax.jit
def pallas_recurrent_scan__ssm_conv_s5__mixer_s_mlp__prompt_kernel(
    A_x: jax.Array,
    A_Lambda_re: jax.Array,
    A_Lambda_im: jax.Array,
    A_B_re: jax.Array,
    A_B_im: jax.Array,
    A_C_re: jax.Array,
    A_C_im: jax.Array,
    A_log_dt: jax.Array,
    A_Dskip: jax.Array,
    B_x: jax.Array,
    B_w1: jax.Array,
    B_w2: jax.Array,
    B_w3: jax.Array,
    B_w4: jax.Array,
):
    x = A_x.reshape(S, D)
    anyspec = pl.BlockSpec(memory_space=pl.ANY)
    out = pl.pallas_call(
        _kernel,
        grid=(NSTEP,),
        in_specs=[anyspec] * 13,
        out_specs=anyspec,
        out_shape=jax.ShapeDtypeStruct((NSTEP, NSEG, SEG, D), f32),
        scratch_shapes=[
            pltpu.VMEM((S, D), bf16),
            pltpu.VMEM((P, D), bf16),
            pltpu.VMEM((P, D), bf16),
            pltpu.VMEM((D, P), bf16),
            pltpu.VMEM((D, P), bf16),
            pltpu.VMEM((D, D), bf16),
            pltpu.VMEM((D, D), bf16),
            pltpu.VMEM((D, F), bf16),
            pltpu.VMEM((F, D), bf16),
            pltpu.SemaphoreType.DMA((11,)),
            pltpu.VMEM((D, 2 * P), bf16),
            pltpu.VMEM((T, P), f32),
            pltpu.VMEM((T, P), f32),
            pltpu.VMEM((8, 8, P), f32),
            pltpu.VMEM((2, 8, P), f32),
            pltpu.VMEM((2, T, D), f32),
            pltpu.VMEM((2, T, D), f32),
            pltpu.VMEM((T, 2 * P), f32),
            pltpu.VMEM((T + 32, D), f32),
            pltpu.VMEM((2, T, D), bf16),
            pltpu.VMEM((2, SEG, NSEG, D), f32),
            pltpu.SemaphoreType.DMA((2,)),
            pltpu.VMEM((T, D), bf16),
            pltpu.VMEM((P,), bf16),
            pltpu.VMEM((P,), bf16),
            pltpu.VMEM((P,), bf16),
            pltpu.VMEM((D,), bf16),
            pltpu.SemaphoreType.DMA((4,)),
        ],
        compiler_params=pltpu.CompilerParams(
            dimension_semantics=("arbitrary",),
            vmem_limit_bytes=100 * 1024 * 1024,
        ),
    )(A_Lambda_re, A_Lambda_im, A_log_dt, A_Dskip,
      x, A_B_re, A_B_im, A_C_re, A_C_im, B_w1, B_w2, B_w3, B_w4)
    return out.reshape(1, S, D)
```
